```python
import os as _os
_os.environ.setdefault("JAX_PLATFORMS", "cpu")
import jax
import jax.numpy as jnp

def _softmax(x, axis=-1):
    return jax.nn.softmax(x, axis=axis)
def _gelu(x):
    return jax.nn.gelu(x, approximate=True)
def _silu(x):
    return jax.nn.silu(x)
def _sigmoid(x):
    return jax.nn.sigmoid(x)
def _layernorm(x, axis=-1, eps=1e-5):
    m = jnp.mean(x, axis=axis, keepdims=True)
    v = jnp.var(x, axis=axis, keepdims=True)
    return (x - m) / jnp.sqrt(v + eps)
def _scatter_add(tgt, idx, src, axis=0):
    return tgt.at[idx].add(src)
def _segment_sum(src, seg, n):
    return jax.ops.segment_sum(src, seg, n)
class _Rng:
    def __init__(self, key):
        self._k = key
    def _next(self):
        self._k, sub = jax.random.split(self._k)
        return sub
    def normal(self, shape):
        return jax.random.normal(self._next(), shape, dtype=jnp.bfloat16)
    def randint(self, lo, hi, shape):
        return jax.random.randint(self._next(), shape, lo, hi, dtype=jnp.int32)
    def uniform(self, shape, lo=0.0, hi=1.0):
        return jax.random.uniform(self._next(), shape, jnp.bfloat16, lo, hi)
    def permutation(self, n):
        return jax.random.permutation(self._next(), n)


kernel_name = 'parallel_sum__softmax_full_mha__moe_arch_mod__prompt'

def setup_inputs():
    _rng = _Rng(jax.random.key(int.from_bytes(__import__("os").urandom(4), "little")))
    _w = (lambda a: (lambda t: t.astype(jnp.bfloat16) if jnp.issubdtype(t.dtype, jnp.floating) else t)(jnp.asarray(a)))
    def _A_setup():
        B, S, D = 1, 2048, 512
        return {
            "x": _w((lambda *s: _rng.normal(s) * 0.05)(B, S, D)),
            "wqkv": _w((lambda *s: _rng.normal(s) * 0.1)(D, 3 * D)),
            "wo": _w((lambda *s: _rng.normal(s) * 0.05)(D, D)),
        }
    _A_in = _A_setup()

    def _B_setup():
        B, S, D, F, C = 1, 2048, 512, 1792, 1
        return {
            "x": _w((lambda *s: _rng.normal(s) * 0.05)(B, S, D)),
            "w_r": _w((lambda *s: _rng.normal(s) * 1.6)(D)),
            "w_gate": _w((lambda *s: _rng.normal(s) * 0.1)(D, F)),
            "w_up": _w((lambda *s: _rng.normal(s) * 0.1)(D, F)),
            "w_down": _w((lambda *s: _rng.normal(s) * 0.1)(F, D)),
        }
    _B_in = _B_setup()

    return {
        "A_x": _A_in["x"],
        "A_wqkv": _A_in["wqkv"],
        "A_wo": _A_in["wo"],
        "B_x": _B_in["x"],
        "B_w_r": _B_in["w_r"],
        "B_w_gate": _B_in["w_gate"],
        "B_w_up": _B_in["w_up"],
        "B_w_down": _B_in["w_down"],
    }

def reference(A_x, A_wqkv, A_wo, B_x, B_w_r, B_w_gate, B_w_up, B_w_down):
    def _A_ref(x, wqkv, wo):
        B, S, D = x.shape
        H = 32; Dh = D // H
        qkv = (lambda x, *d: x.transpose(*d))((x @ wqkv).reshape(B, S, 3, H, Dh), 2, 0, 3, 1, 4)
        q, k, v = qkv[0], qkv[1], qkv[2]
        scale = Dh ** -0.5
        scores = jnp.einsum("bhqd,bhkd->bhqk", q, k) * scale
        p = _softmax(scores, axis=-1)
        o = jnp.einsum("bhqk,bhkd->bhqd", p, v)
        return (lambda x, *d: x.transpose(*d))(o, 0, 2, 1, 3).reshape(B, S, D) @ wo

    def _B_ref(x, w_r, w_gate, w_up, w_down):
        B, S, D = x.shape
        C = 1
        r = x @ w_r
        idx = jnp.argsort(-r, axis=-1)[:, :C]
        idx_e = jnp.repeat(idx.reshape(B, C, 1), D, axis=2)
        x_sel = jnp.take_along_axis(x, idx_e, axis=1)
        g = _silu(x_sel @ w_gate)
        u = x_sel @ w_up
        y = (g * u) @ w_down
        r_sel = _sigmoid(jnp.take_along_axis(r, idx, axis=1))
        y = y * r_sel.reshape(B, C, 1)
        b_off = (jnp.arange(B) * S).reshape(B, 1)
        flat_idx = (idx + b_off).reshape(B * C)
        zero = (x * 0.0).reshape(B * S, D)
        upd = _scatter_add(zero, flat_idx, y.reshape(B * C, D), axis=0)
        return x + upd.reshape(B, S, D)

    x = A_x
    xn = _layernorm(x, axis=-1)
    return x + _A_ref(xn, A_wqkv, A_wo) + _B_ref(xn, B_w_r, B_w_gate, B_w_up, B_w_down)
```

```python
import functools
import math

import jax
import jax.numpy as jnp
import numpy as np
import jax.experimental.pallas as pl
import jax.experimental.pallas.tpu as pltpu

_H = 32
_LANES = 128
_TQ = 512
_TK = 256

_F32 = jnp.float32
_BF16 = jnp.bfloat16


def _bf(x):
    return x.astype(_BF16).astype(_F32)


def _kernel(x_ref, wqkv_ref, wo_ref, wr_ref, wg_hbm, wu_hbm, wd_hbm,
            o_ref,
            xn_ref, q_ref, k_ref, vt_ref, s_ref, qm_ref, ot_ref, y_ref, idx_ref,
            wg_ref, wu_ref, wd_ref, sems,
            *, S, D, F, TQ, TK):
    H = _H
    DH = D // H
    HPG = _LANES // DH
    NK = S // TK
    step = pl.program_id(0)

    @pl.when(step == 0)
    def _phase1():
        cg = pltpu.make_async_copy(wg_hbm, wg_ref, sems.at[0])
        cu = pltpu.make_async_copy(wu_hbm, wu_ref, sems.at[1])
        cd = pltpu.make_async_copy(wd_hbm, wd_ref, sems.at[2])
        cg.start()
        cu.start()
        cd.start()

        eps_b = float(np.asarray(1e-5, dtype=jnp.bfloat16).astype(np.float32))
        qscale = (DH ** -0.5) * math.log2(math.e)

        RB = 256

        def ln_body(i, carry):
            r0 = pl.multiple_of(i * RB, RB)
            xf = x_ref[pl.ds(r0, RB), :].astype(_F32)
            mean = jnp.sum(xf, axis=-1, keepdims=True) * (1.0 / D)
            cen = xf - mean
            var = jnp.sum(cen * cen, axis=-1, keepdims=True) * (1.0 / D)
            m_b = _bf(mean)
            v_b = _bf(var)
            d = _bf(xf - m_b)
            sd = _bf(jnp.sqrt(_bf(v_b + eps_b)))
            xn = (d / sd).astype(_BF16)
            xn_ref[pl.ds(r0, RB), :] = xn
            qk = jnp.dot(xn, wqkv_ref[:, 0:2 * D], preferred_element_type=_F32)
            q_ref[pl.ds(r0, RB), :] = (qk[:, 0:D] * qscale).astype(_BF16)
            k_ref[pl.ds(r0, RB), :] = qk[:, D:2 * D].astype(_BF16)
            return carry

        jax.lax.fori_loop(0, S // RB, ln_body, 0)

        wvt = wqkv_ref[:, 2 * D:3 * D].astype(_F32).T.astype(_BF16)
        wr_rows = jnp.broadcast_to(wr_ref[...], (16, D))
        lhs = jnp.concatenate([wvt, wr_rows], axis=0)
        vt = jax.lax.dot_general(lhs, xn_ref[...], (((1,), (1,)), ((), ())),
                                 preferred_element_type=_F32)
        vt_ref[...] = vt[0:D, :].astype(_BF16)
        r = _bf(vt[D:D + 8, :])
        rmax = jnp.max(r, axis=1, keepdims=True)
        lane = jax.lax.broadcasted_iota(jnp.int32, (8, S), 1)
        idx = jnp.min(jnp.where(r == rmax, lane, S), axis=1, keepdims=True)
        idx_ref[...] = idx
        lane16 = jax.lax.broadcasted_iota(jnp.int32, (16, S), 1)
        onehot = jnp.where(lane16 == idx[0:1, :], 1.0, 0.0).astype(_BF16)
        x_sel = jnp.dot(onehot, xn_ref[...], preferred_element_type=_F32).astype(_BF16)

        cg.wait()
        cu.wait()
        cd.wait()
        g = _bf(jnp.dot(x_sel, wg_ref[...], preferred_element_type=_F32))
        g = _bf(g * jax.nn.sigmoid(g))
        u = _bf(jnp.dot(x_sel, wu_ref[...], preferred_element_type=_F32))
        gu = (g * u).astype(_BF16)
        y = _bf(jnp.dot(gu, wd_ref[...], preferred_element_type=_F32))
        r_sel = _bf(jax.nn.sigmoid(rmax[0:1, :]))
        y_ref[...] = _bf(y[0:8, :] * r_sel)

    q0 = pl.multiple_of(step * TQ, TQ)
    lane_head = jax.lax.broadcasted_iota(jnp.int32, (TQ, _LANES), 1) // DH

    def make_qm(h, slot):
        g0 = pl.multiple_of((h // HPG) * _LANES, _LANES)
        qg = q_ref[pl.ds(q0, TQ), pl.ds(g0, _LANES)]
        qm_ref[slot] = jnp.where(lane_head == (h % HPG), qg, jnp.zeros_like(qg))

    def stage_a(h, slot, kc, m8):
        g0 = pl.multiple_of((h // HPG) * _LANES, _LANES)
        k0 = pl.multiple_of(kc * TK, TK)
        kc_blk = k_ref[pl.ds(k0, TK), pl.ds(g0, _LANES)]
        s = jax.lax.dot_general(kc_blk, qm_ref[slot], (((1,), (1,)), ((), ())),
                                preferred_element_type=_F32)
        s_ref[slot, pl.ds(k0, TK), :] = s
        return jnp.maximum(m8, jnp.max(s.reshape(TK // 8, 8, TQ), axis=0))

    def stage_b(h, slot, kc, m, l8, acc):
        k0 = pl.multiple_of(kc * TK, TK)
        h0 = pl.multiple_of(h * DH, DH)
        p = jnp.exp2(s_ref[slot, pl.ds(k0, TK), :] - m)
        l8 = l8 + jnp.sum(p.reshape(TK // 8, 8, TQ), axis=0)
        acc = acc + jnp.dot(vt_ref[pl.ds(h0, DH), pl.ds(k0, TK)], p.astype(_BF16),
                            preferred_element_type=_F32)
        return l8, acc

    def finish_b(h, l8, acc):
        h0 = pl.multiple_of(h * DH, DH)
        l = jnp.sum(l8, axis=0, keepdims=True)
        ot_ref[pl.ds(h0, DH), :] = acc / l

    neg = jnp.full((8, TQ), -jnp.inf, _F32)
    zl = jnp.zeros((8, TQ), _F32)
    za = jnp.zeros((DH, TQ), _F32)

    make_qm(0, 0)
    m8 = jax.lax.fori_loop(0, NK, lambda kc, m8: stage_a(0, 0, kc, m8), neg)
    m_first = jnp.max(m8, axis=0, keepdims=True)

    def head_body(h, m_cur):
        slot = h % 2
        nslot = 1 - slot
        make_qm(h + 1, nslot)

        def chunk(kc, carry):
            m8, l8, acc = carry
            m8 = stage_a(h + 1, nslot, kc, m8)
            l8, acc = stage_b(h, slot, kc, m_cur, l8, acc)
            return m8, l8, acc

        m8, l8, acc = jax.lax.fori_loop(0, NK, chunk, (neg, zl, za))
        finish_b(h, l8, acc)
        return jnp.max(m8, axis=0, keepdims=True)

    m_last = jax.lax.fori_loop(0, H - 1, head_body, m_first)

    def last_chunk(kc, carry):
        l8, acc = carry
        return stage_b(H - 1, (H - 1) % 2, kc, m_last, l8, acc)

    l8, acc = jax.lax.fori_loop(0, NK, last_chunk, (zl, za))
    finish_b(H - 1, l8, acc)

    o = ot_ref[...].T.astype(_BF16)
    attn = _bf(jnp.dot(o, wo_ref[...], preferred_element_type=_F32))
    xf = x_ref[pl.ds(q0, TQ), :].astype(_F32)
    xnf = xn_ref[pl.ds(q0, TQ), :].astype(_F32)
    row = jax.lax.broadcasted_iota(jnp.int32, (TQ, D), 0) + q0
    upd = jnp.where(row == idx_ref[0:1, :], y_ref[0:1, :], 0.0)
    o_ref[...] = (_bf(xf + attn) + _bf(xnf + upd)).astype(o_ref.dtype)


@jax.jit
def pallas_parallel_sum__softmax_full_mha__moe_arch_mod__prompt_kernel(
    A_x: jax.Array,
    A_wqkv: jax.Array,
    A_wo: jax.Array,
    B_x: jax.Array,
    B_w_r: jax.Array,
    B_w_gate: jax.Array,
    B_w_up: jax.Array,
    B_w_down: jax.Array,
):
    B, S, D = A_x.shape
    assert B == 1
    F = B_w_gate.shape[1]
    TQ, TK = _TQ, _TK
    x2 = A_x.reshape(S, D)
    wr2 = B_w_r.reshape(1, D)

    kern = functools.partial(_kernel, S=S, D=D, F=F, TQ=TQ, TK=TK)
    full = lambda shape: pl.BlockSpec(shape, lambda i: (0,) * len(shape))
    out = pl.pallas_call(
        kern,
        grid=(S // TQ,),
        in_specs=[
            full((S, D)),
            full((D, 3 * D)),
            full((D, D)),
            full((1, D)),
            pl.BlockSpec(memory_space=pl.ANY),
            pl.BlockSpec(memory_space=pl.ANY),
            pl.BlockSpec(memory_space=pl.ANY),
        ],
        out_specs=pl.BlockSpec((TQ, D), lambda i: (i, 0)),
        out_shape=jax.ShapeDtypeStruct((S, D), A_x.dtype),
        scratch_shapes=[
            pltpu.VMEM((S, D), _BF16),
            pltpu.VMEM((S, D), _BF16),
            pltpu.VMEM((S, D), _BF16),
            pltpu.VMEM((D, S), _BF16),
            pltpu.VMEM((2, S, TQ), _F32),
            pltpu.VMEM((2, TQ, _LANES), _BF16),
            pltpu.VMEM((D, TQ), _F32),
            pltpu.VMEM((8, D), _F32),
            pltpu.VMEM((8, 1), jnp.int32),
            pltpu.VMEM((D, F), _BF16),
            pltpu.VMEM((D, F), _BF16),
            pltpu.VMEM((F, D), _BF16),
            pltpu.SemaphoreType.DMA((3,)),
        ],
        compiler_params=pltpu.CompilerParams(
            dimension_semantics=("arbitrary",),
            vmem_limit_bytes=100 * 1024 * 1024,
        ),
    )(x2, A_wqkv, A_wo, wr2, B_w_gate, B_w_up, B_w_down)
    return out.reshape(B, S, D)
```

```python
import functools
import math

import jax
import jax.numpy as jnp
import numpy as np
import jax.experimental.pallas as pl
import jax.experimental.pallas.tpu as pltpu

_H = 32
_LANES = 128
_TQ = 512
_TK = 128
_G = 4
_OS = 128
_NSIDE = 8
_RB = 256

_F32 = jnp.float32
_BF16 = jnp.bfloat16


def _bf(x):
    return x.astype(_BF16).astype(_F32)


def _kernel(x_hbm, wqkv_hbm, wo_hbm, wr_ref, wg_hbm, wu_hbm, wd_hbm,
            o_hbm,
            x_ref, wq_ref, wk_ref, wv_ref, wo_ref, wg_ref, wu_ref, wd_ref,
            wt_ref, xn_ref, qt_ref, kh_ref, vt_ref, r_ref, ot_ref,
            on_ref, ob_ref, sems, xsems, osems, *s_refs_all,
            S, D, F, TQ, TK, RB):
    H = _H
    DH = D // H
    HPG = _LANES // DH
    NK = S // TK
    NQ = S // TQ
    NRB = S // RB
    NITEMS = NQ * H

    def x_copy(i):
        return pltpu.make_async_copy(x_hbm.at[pl.ds(i * RB, RB), :],
                                     x_ref.at[pl.ds(i * RB, RB), :], xsems.at[i])

    cwq = pltpu.make_async_copy(wqkv_hbm.at[:, pl.ds(0, D)], wq_ref, sems.at[0])
    cwk = pltpu.make_async_copy(wqkv_hbm.at[:, pl.ds(D, D)], wk_ref, sems.at[1])
    cwv = pltpu.make_async_copy(wqkv_hbm.at[:, pl.ds(2 * D, D)], wv_ref, sems.at[2])
    co = pltpu.make_async_copy(wo_hbm, wo_ref, sems.at[3])
    cg = pltpu.make_async_copy(wg_hbm, wg_ref, sems.at[4])
    cu = pltpu.make_async_copy(wu_hbm, wu_ref, sems.at[5])
    cd = pltpu.make_async_copy(wd_hbm, wd_ref, sems.at[6])
    x_copy(0).start()
    x_copy(1).start()
    cwk.start()
    x_copy(2).start()
    cwq.start()
    cwv.start()
    for i in range(3, NRB):
        x_copy(i).start()

    eps_b = float(np.asarray(1e-5, dtype=jnp.bfloat16).astype(np.float32))
    qscale = (DH ** -0.5) * math.log2(math.e)

    def ln_rows(r0):
        xf = x_ref[pl.ds(r0, RB), :].astype(_F32)
        mean = jnp.sum(xf, axis=-1, keepdims=True) * (1.0 / D)
        cen = xf - mean
        var = jnp.sum(cen * cen, axis=-1, keepdims=True) * (1.0 / D)
        m_b = _bf(mean)
        v_b = _bf(var)
        d = _bf(xf - m_b)
        sd = _bf(jnp.sqrt(_bf(v_b + eps_b)))
        xn_ref[pl.ds(r0, RB), :] = (d / sd).astype(_BF16)

    def k_rows(r0):
        xn = xn_ref[pl.ds(r0, RB), :]
        kk = jnp.dot(xn, wk_ref[...], preferred_element_type=_F32).astype(_BF16)
        kw = pltpu.bitcast(kk, jnp.uint32)
        for gi in range(D // _LANES):
            kg = kw[:, gi * _LANES:(gi + 1) * _LANES]
            for j in range(HPG):
                kr = kg if j == 0 else pltpu.roll(kg, _LANES - j * DH, 1)
                kh_ref[gi * HPG + j, pl.ds(r0 // 2, RB // 2), :] = kr

    def qv_rows(r0):
        t = jax.lax.dot_general(wt_ref[...], xn_ref[pl.ds(r0, RB), :], (((1,), (1,)), ((), ())),
                                preferred_element_type=_F32)
        qt_ref[:, pl.ds(r0, RB)] = pltpu.bitcast((t[0:D, :] * qscale).astype(_BF16), jnp.uint32)
        vt_ref[:, pl.ds(r0, RB)] = pltpu.bitcast(t[D:2 * D, :].astype(_BF16), jnp.uint32)
        r_ref[:, pl.ds(r0, RB)] = _bf(t[2 * D:2 * D + 8, :])

    x_copy(0).wait()
    ln_rows(0)
    x_copy(1).wait()
    ln_rows(RB)
    cwk.wait()
    x_copy(2).wait()
    k_rows(0)
    ln_rows(2 * RB)
    k_rows(RB)
    cwq.wait()
    cwv.wait()
    x_copy(3).wait()
    wt_ref[0:D, :] = wq_ref[...].astype(_F32).T.astype(_BF16)
    k_rows(2 * RB)
    wt_ref[D:2 * D, :] = wv_ref[...].astype(_F32).T.astype(_BF16)
    wt_ref[2 * D:2 * D + 16, :] = jnp.broadcast_to(wr_ref[...], (16, D))
    ln_rows(3 * RB)
    for i in range(4, NRB):
        x_copy(i).wait()
    co.start()
    cg.start()
    cu.start()
    cd.start()
    for i in range(NRB):
        if i + 4 < NRB:
            ln_rows((i + 4) * RB)
        qv_rows(i * RB)
        if i + 3 < NRB:
            k_rows((i + 3) * RB)

    rt = {}
    FC = 2 * _LANES
    NFC = F // FC

    def rt_select():
        r = r_ref[...]
        rmax = jnp.max(r, axis=1, keepdims=True)
        lane = jax.lax.broadcasted_iota(jnp.int32, (8, S), 1)
        idx = jnp.min(jnp.where(r == rmax, lane, S))
        g0 = pl.multiple_of((idx // 16) * 16, 16)
        rt["g0"] = g0
        rt["sub"] = idx - g0
        rt["r_sel"] = _bf(jax.nn.sigmoid(rmax[0:1, :]))
        rt["x_sel"] = xn_ref[pl.ds(g0, 16), :]
        rt["y"] = jnp.zeros((16, D), _F32)

    def rt_ffn(i):
        c0 = i * FC
        g = _bf(jnp.dot(rt["x_sel"], wg_ref[:, c0:c0 + FC], preferred_element_type=_F32))
        g = _bf(g * jax.nn.sigmoid(g))
        u = _bf(jnp.dot(rt["x_sel"], wu_ref[:, c0:c0 + FC], preferred_element_type=_F32))
        rt["gu", i] = (g * u).astype(_BF16)

    def rt_down(i):
        c0 = i * FC
        rt["y"] = rt["y"] + jnp.dot(rt.pop(("gu", i)), wd_ref[c0:c0 + FC, :],
                                    preferred_element_type=_F32)

    def rt_final():
        sub = jax.lax.broadcasted_iota(jnp.int32, (16, D), 0)
        upd = jnp.where(sub == rt["sub"], _bf(_bf(rt["y"]) * rt["r_sel"]), 0.0)
        xn_ref[pl.ds(rt["g0"], 16), :] = (rt["x_sel"].astype(_F32) + upd).astype(_BF16)

    G = _G
    s_sets = (s_refs_all[0:G], s_refs_all[G:2 * G])
    HW = DH // 2

    def stage_a(item, sref, kc, m8):
        h = item % H
        q0 = pl.multiple_of((item // H) * TQ, TQ)
        h0 = pl.multiple_of(h * HW, HW)
        k0 = kc * TK
        kc_blk = pltpu.bitcast(kh_ref[h, pl.ds(k0 // 2, TK // 2), :], _BF16)[:, 0:DH]
        qw = pltpu.bitcast(qt_ref[pl.ds(h0, HW), pl.ds(q0, TQ)], _BF16)
        s = jnp.dot(kc_blk, qw, preferred_element_type=_F32)
        sref[pl.ds(k0, TK), :] = s
        return jnp.maximum(m8, jnp.max(s.reshape(TK // 8, 8, TQ), axis=0))

    def stage_b(item, sref, kc, m, l8, acc):
        k0 = kc * TK
        h0 = pl.multiple_of((item % H) * HW, HW)
        pieces = []
        for r in range(TK // 16):
            pa = jnp.exp2(sref[pl.ds(k0 + 16 * r, 8), :] - m)
            pb = jnp.exp2(sref[pl.ds(k0 + 16 * r + 8, 8), :] - m)
            l8 = (l8 + pa) + pb
            pieces += [pa, pb]
        p = jnp.concatenate(pieces, axis=0).astype(_BF16)
        vw = pltpu.bitcast(vt_ref[pl.ds(h0, HW), pl.ds(k0, TK)], _BF16)
        acc = acc + jnp.dot(vw, p, preferred_element_type=_F32)
        return l8, acc

    def finish(item, l8, acc):
        qt = item // H
        h0 = pl.multiple_of((item % H) * DH, DH)
        l = jnp.sum(l8, axis=0, keepdims=True)
        ot_ref[qt, pl.ds(h0, DH), :] = acc / l

    neg = jnp.full((8, TQ), -jnp.inf, _F32)
    zl = jnp.zeros((8, TQ), _F32)
    za = jnp.zeros((DH, TQ), _F32)

    def bmax(m8):
        return jnp.broadcast_to(jnp.max(m8, axis=0, keepdims=True), (8, TQ))

    def block(base, par, ms, do_a=True, do_b=True, side=None):
        new_ms = []
        m8 = l8 = acc = None
        for t in range(G * NK):
            g, c = divmod(t, NK)
            if do_a:
                if c == 0:
                    m8 = neg
                m8 = stage_a(base + G + g, s_sets[1 - par][g], c, m8)
                if c == NK - 1:
                    new_ms.append(bmax(m8))
            if do_b:
                if c == 0:
                    l8, acc = zl, za
                l8, acc = stage_b(base + g, s_sets[par][g], c, ms[g], l8, acc)
                if c == NK - 1:
                    finish(base + g, l8, acc)
            if side is not None:
                for task in side.get(t, ()):
                    task()
        return tuple(new_ms)

    NB = NITEMS // G
    cg.wait()
    cu.wait()
    cd.wait()
    side = {0: [rt_select]}
    stride = (G * NK - 4) // (NFC + 1)
    for i in range(NFC):
        side.setdefault(2 + i * stride, []).append(functools.partial(rt_ffn, i))
        side.setdefault(2 + (i + 1) * stride, []).append(functools.partial(rt_down, i))
    side.setdefault(G * NK - 1, []).append(rt_final)
    ms = block(-G, 1, None, do_b=False, side=side)

    def body(j, ms):
        return jax.lax.cond(j % 2 == 0,
                            lambda ms: block(j * G, 0, ms),
                            lambda ms: block(j * G, 1, ms), ms)

    ms = jax.lax.fori_loop(0, NB - 1, body, ms)

    co.wait()

    def o_copy(t):
        return pltpu.make_async_copy(ob_ref.at[t], o_hbm.at[pl.ds(t * TQ, TQ), :], osems.at[t])

    def o_copy_slice(j):
        t = NQ - 1
        return pltpu.make_async_copy(ob_ref.at[t, pl.ds(j * _OS, _OS), :],
                                     o_hbm.at[pl.ds(t * TQ + j * _OS, _OS), :], osems.at[t + j])

    OS = _OS
    NS = TQ // OS
    NC = D // _LANES

    def out_prep(t, j):
        o = ot_ref[t, :, pl.ds(j * OS, OS)].T.astype(_BF16)
        on_ref[pl.ds((t * TQ + j * OS) // 2, OS // 2), :] = pltpu.bitcast(o, jnp.uint32)

    def out_piece(t, j, n):
        q0 = t * TQ + j * OS
        c0 = n * _LANES
        o = pltpu.bitcast(on_ref[pl.ds(q0 // 2, OS // 2), :], _BF16)
        attn = jnp.dot(o, wo_ref[:, c0:c0 + _LANES], preferred_element_type=_F32)
        xf = x_ref[pl.ds(q0, OS), c0:c0 + _LANES].astype(_F32)
        xnf = xn_ref[pl.ds(q0, OS), c0:c0 + _LANES].astype(_F32)
        ob_ref[t, pl.ds(j * OS, OS), c0:c0 + _LANES] = ((xf + attn) + xnf).astype(ob_ref.dtype)

    slices = [(t, j) for t in range(NQ - 1) for j in range(NS)]
    tasks = []
    for i, (t, j) in enumerate(slices):
        for n in range(NC):
            tk = [functools.partial(out_piece, t, j, n)]
            if n == 0 and i + 1 < len(slices):
                tk.append(functools.partial(out_prep, *slices[i + 1]))
            tasks.append(tk)
    out_prep(*slices[0])
    n_side = min(len(tasks), G * NK - 1)
    side = {1 + (n * (G * NK - 1)) // n_side: tasks[n] for n in range(n_side)}
    block((NB - 1) * G, (NB - 1) % 2, ms, do_a=False, side=side)
    for tk in tasks[n_side:]:
        for task in tk:
            task()
    for t in range(NQ - 1):
        o_copy(t).start()
    for j in range(NS):
        out_prep(NQ - 1, j)
    for j in range(NS):
        for n in range(NC):
            out_piece(NQ - 1, j, n)
        o_copy_slice(j).start()
    for t in range(NQ - 1):
        o_copy(t).wait()
    for j in range(NS):
        o_copy_slice(j).wait()


@jax.jit
def pallas_parallel_sum__softmax_full_mha__moe_arch_mod__prompt_kernel(
    A_x: jax.Array,
    A_wqkv: jax.Array,
    A_wo: jax.Array,
    B_x: jax.Array,
    B_w_r: jax.Array,
    B_w_gate: jax.Array,
    B_w_up: jax.Array,
    B_w_down: jax.Array,
):
    B, S, D = A_x.shape
    assert B == 1
    F = B_w_gate.shape[1]
    TQ, TK, RB = _TQ, _TK, _RB
    NQ = S // TQ
    x2 = A_x.reshape(S, D)
    wr2 = B_w_r.reshape(1, D)

    kern = functools.partial(_kernel, S=S, D=D, F=F, TQ=TQ, TK=TK, RB=RB)
    hbm = pl.BlockSpec(memory_space=pl.ANY)
    out = pl.pallas_call(
        kern,
        in_specs=[hbm, hbm, hbm, pl.BlockSpec(memory_space=pltpu.VMEM), hbm, hbm, hbm],
        out_specs=hbm,
        out_shape=jax.ShapeDtypeStruct((S, D), A_x.dtype),
        scratch_shapes=[
            pltpu.VMEM((S, D), _BF16),
            pltpu.VMEM((D, D), _BF16),
            pltpu.VMEM((D, D), _BF16),
            pltpu.VMEM((D, D), _BF16),
            pltpu.VMEM((D, D), _BF16),
            pltpu.VMEM((D, F), _BF16),
            pltpu.VMEM((D, F), _BF16),
            pltpu.VMEM((F, D), _BF16),
            pltpu.VMEM((2 * D + 16, D), _BF16),
            pltpu.VMEM((S, D), _BF16),
            pltpu.VMEM((D // 2, S), jnp.uint32),
            pltpu.VMEM((_H, S // 2, _LANES), jnp.uint32),
            pltpu.VMEM((D // 2, S), jnp.uint32),
            pltpu.VMEM((8, S), _F32),
            pltpu.VMEM((NQ, D, TQ), _F32),
            pltpu.VMEM((S // 2, D), jnp.uint32),
            pltpu.VMEM((NQ, TQ, D), _BF16),
            pltpu.SemaphoreType.DMA((7,)),
            pltpu.SemaphoreType.DMA((S // RB,)),
            pltpu.SemaphoreType.DMA((NQ - 1 + TQ // _OS,)),
        ] + [pltpu.VMEM((S, TQ), _F32) for _ in range(2 * _G)],
        compiler_params=pltpu.CompilerParams(
            vmem_limit_bytes=110 * 1024 * 1024,
        ),
    )(x2, A_wqkv, A_wo, wr2, B_w_gate, B_w_up, B_w_down)
    return out.reshape(B, S, D)
```

```python
import functools
import math

import jax
import jax.numpy as jnp
import numpy as np
import jax.experimental.pallas as pl
import jax.experimental.pallas.tpu as pltpu

_H = 32
_LANES = 128
_TQ = 256
_TK = 128
_G = 8
_OS = 128
_RB = 256

_F32 = jnp.float32
_BF16 = jnp.bfloat16


def _bf(x):
    return x.astype(_BF16).astype(_F32)


def _kernel(x_hbm, wqkv_hbm, wo_hbm, wr_ref, wg_hbm, wu_hbm, wd_hbm,
            o_hbm,
            x_ref, wq_ref, wk_ref, wv_ref, wo_ref, wg_ref, wu_ref, wd_ref,
            wt_ref, xn_ref, qt_ref, kh_ref, vt_ref, r_ref, ot_ref,
            on_ref, ob_ref, sems, xsems, osems, *s_refs_all,
            S, D, F, TQ, TK, RB):
    H = _H
    DH = D // H
    HPG = _LANES // DH
    NK = S // TK
    NQ = S // TQ
    NRB = S // RB
    NITEMS = NQ * H

    def x_copy(i):
        return pltpu.make_async_copy(x_hbm.at[pl.ds(i * RB, RB), :],
                                     x_ref.at[pl.ds(i * RB, RB), :], xsems.at[i])

    cwq = pltpu.make_async_copy(wqkv_hbm.at[:, pl.ds(0, D)], wq_ref, sems.at[0])
    cwk = pltpu.make_async_copy(wqkv_hbm.at[:, pl.ds(D, D)], wk_ref, sems.at[1])
    cwv = pltpu.make_async_copy(wqkv_hbm.at[:, pl.ds(2 * D, D)], wv_ref, sems.at[2])
    co = pltpu.make_async_copy(wo_hbm, wo_ref, sems.at[3])
    cg = pltpu.make_async_copy(wg_hbm, wg_ref, sems.at[4])
    cu = pltpu.make_async_copy(wu_hbm, wu_ref, sems.at[5])
    cd = pltpu.make_async_copy(wd_hbm, wd_ref, sems.at[6])
    x_copy(0).start()
    cwk.start()
    cwq.start()
    cwv.start()
    for i in range(1, NRB):
        x_copy(i).start()

    eps_b = float(np.asarray(1e-5, dtype=jnp.bfloat16).astype(np.float32))
    qscale = (DH ** -0.5) * math.log2(math.e)

    def ln_rows(r0):
        xf = x_ref[pl.ds(r0, RB), :].astype(_F32)
        mean = jnp.sum(xf, axis=-1, keepdims=True) * (1.0 / D)
        cen = xf - mean
        var = jnp.sum(cen * cen, axis=-1, keepdims=True) * (1.0 / D)
        m_b = _bf(mean)
        v_b = _bf(var)
        d = _bf(xf - m_b)
        sd = _bf(jnp.sqrt(_bf(v_b + eps_b)))
        xn_ref[pl.ds(r0, RB), :] = (d / sd).astype(_BF16)

    def k_rows(r0):
        xn = xn_ref[pl.ds(r0, RB), :]
        kk = jnp.dot(xn, wk_ref[...], preferred_element_type=_F32).astype(_BF16)
        kw = pltpu.bitcast(kk, jnp.uint32)
        for gi in range(D // _LANES):
            kg = kw[:, gi * _LANES:(gi + 1) * _LANES]
            for j in range(HPG):
                kr = kg if j == 0 else pltpu.roll(kg, _LANES - j * DH, 1)
                kh_ref[gi * HPG + j, pl.ds(r0 // 2, RB // 2), :] = kr

    def qv_rows(r0):
        t = jax.lax.dot_general(wt_ref[...], xn_ref[pl.ds(r0, RB), :], (((1,), (1,)), ((), ())),
                                preferred_element_type=_F32)
        qt_ref[:, pl.ds(r0, RB)] = pltpu.bitcast((t[0:D, :] * qscale).astype(_BF16), jnp.uint32)
        vt_ref[:, pl.ds(r0, RB)] = pltpu.bitcast(t[D:2 * D, :].astype(_BF16), jnp.uint32)
        r_ref[:, pl.ds(r0, RB)] = _bf(t[2 * D:2 * D + 8, :])

    x_copy(0).wait()
    ln_rows(0)
    cwk.wait()
    cwq.wait()
    wt_ref[0:D, :] = wq_ref[...].astype(_F32).T.astype(_BF16)
    k_rows(0)
    cwv.wait()
    x_copy(1).wait()
    wt_ref[D:2 * D, :] = wv_ref[...].astype(_F32).T.astype(_BF16)
    wt_ref[2 * D:2 * D + 16, :] = jnp.broadcast_to(
        wr_ref[...].astype(_F32).reshape(1, D), (16, D)).astype(_BF16)
    ln_rows(RB)
    qv_rows(0)
    x_copy(2).wait()
    x_copy(3).wait()
    ln_rows(2 * RB)
    k_rows(RB)
    ln_rows(3 * RB)
    qv_rows(RB)
    for i in range(4, NRB):
        x_copy(i).wait()
    co.start()
    cg.start()
    cu.start()
    cd.start()
    for i in range(2, NRB):
        if i + 2 < NRB:
            ln_rows((i + 2) * RB)
        k_rows(i * RB)
        qv_rows(i * RB)

    rt = {}
    FC = 2 * _LANES
    NFC = F // FC

    def rt_select():
        r = r_ref[...]
        rmax = jnp.max(r, axis=1, keepdims=True)
        lane = jax.lax.broadcasted_iota(jnp.int32, (8, S), 1)
        idx = jnp.min(jnp.where(r == rmax, lane, S - 1))
        g0 = pl.multiple_of((idx // 16) * 16, 16)
        rt["g0"] = g0
        rt["sub"] = idx - g0
        rt["r_sel"] = _bf(jax.nn.sigmoid(rmax[0:1, :]))
        rt["x_sel"] = xn_ref[pl.ds(g0, 16), :]
        rt["y"] = jnp.zeros((16, D), _F32)

    def rt_ffn(i):
        c0 = i * FC
        g = _bf(jnp.dot(rt["x_sel"], wg_ref[:, c0:c0 + FC], preferred_element_type=_F32))
        g = _bf(g * jax.nn.sigmoid(g))
        u = _bf(jnp.dot(rt["x_sel"], wu_ref[:, c0:c0 + FC], preferred_element_type=_F32))
        rt["gu", i] = (g * u).astype(_BF16)

    def rt_down(i):
        c0 = i * FC
        rt["y"] = rt["y"] + jnp.dot(rt.pop(("gu", i)), wd_ref[c0:c0 + FC, :],
                                    preferred_element_type=_F32)

    def rt_final():
        sub = jax.lax.broadcasted_iota(jnp.int32, (16, D), 0)
        upd = jnp.where(sub == rt["sub"], _bf(_bf(rt["y"]) * rt["r_sel"]), 0.0)
        xn_ref[pl.ds(rt["g0"], 16), :] = (rt["x_sel"].astype(_F32) + upd).astype(_BF16)

    G = _G
    HW = DH // 2

    def stage_a(item, sref, kc, m8):
        h = item % H
        q0 = pl.multiple_of((item // H) * TQ, TQ)
        h0 = pl.multiple_of(h * HW, HW)
        k0 = kc * TK
        kc_blk = pltpu.bitcast(kh_ref[h, pl.ds(k0 // 2, TK // 2), :], _BF16)[:, 0:DH]
        qw = pltpu.bitcast(qt_ref[pl.ds(h0, HW), pl.ds(q0, TQ)], _BF16)
        s = jnp.dot(kc_blk, qw, preferred_element_type=_F32)
        sref[pl.ds(k0, TK), :] = s
        return jnp.maximum(m8, jnp.max(s.reshape(TK // 8, 8, TQ), axis=0))

    def stage_b(item, sref, kc, m, l8, acc):
        k0 = kc * TK
        h0 = pl.multiple_of((item % H) * HW, HW)
        pieces = []
        for r in range(TK // 16):
            pa = jnp.exp2(sref[pl.ds(k0 + 16 * r, 8), :] - m)
            pb = jnp.exp2(sref[pl.ds(k0 + 16 * r + 8, 8), :] - m)
            l8 = (l8 + pa) + pb
            pieces += [pa, pb]
        p = jnp.concatenate(pieces, axis=0).astype(_BF16)
        vw = pltpu.bitcast(vt_ref[pl.ds(h0, HW), pl.ds(k0, TK)], _BF16)
        acc = acc + jnp.dot(vw, p, preferred_element_type=_F32)
        return l8, acc

    def finish(item, l8, acc):
        qt = item // H
        h0 = pl.multiple_of((item % H) * DH, DH)
        l = jnp.sum(l8, axis=0, keepdims=True)
        ot_ref[qt, pl.ds(h0, DH), :] = acc / l

    neg = jnp.full((8, TQ), -jnp.inf, _F32)
    zl = jnp.zeros((8, TQ), _F32)
    za = jnp.zeros((DH, TQ), _F32)

    def bmax(m8):
        return jnp.broadcast_to(jnp.max(m8, axis=0, keepdims=True), (8, TQ))

    def block(base, ms, do_a=True, do_b=True, side=None):
        new_ms = []
        m8 = l8 = acc = None
        for t in range(G * NK):
            g, c = divmod(t, NK)
            if do_b:
                if c == 0:
                    l8, acc = zl, za
                l8, acc = stage_b(base + g, s_refs_all[g], c, ms[g], l8, acc)
                if c == NK - 1:
                    finish(base + g, l8, acc)
            if do_a:
                if c == 0:
                    m8 = neg
                m8 = stage_a(base + G + g, s_refs_all[g], c, m8)
                if c == NK - 1:
                    new_ms.append(bmax(m8))
            if side is not None:
                for task in side.get(t, ()):
                    task()
        return tuple(new_ms)

    NB = NITEMS // G
    cg.wait()
    cu.wait()
    cd.wait()
    side = {0: [rt_select]}
    stride = (G * NK - 4) // (NFC + 1)
    for i in range(NFC):
        side.setdefault(2 + i * stride, []).append(functools.partial(rt_ffn, i))
        side.setdefault(2 + (i + 1) * stride, []).append(functools.partial(rt_down, i))
    side.setdefault(G * NK - 1, []).append(rt_final)
    ms = block(-G, None, do_b=False, side=side)

    ms = jax.lax.fori_loop(0, NB - 1, lambda j, ms: block(j * G, ms), ms)

    co.wait()

    def o_copy(t):
        return pltpu.make_async_copy(ob_ref.at[t], o_hbm.at[pl.ds(t * TQ, TQ), :], osems.at[t])

    def o_copy_slice(j):
        t = NQ - 1
        return pltpu.make_async_copy(ob_ref.at[t, pl.ds(j * _OS, _OS), :],
                                     o_hbm.at[pl.ds(t * TQ + j * _OS, _OS), :], osems.at[t + j])

    OS = _OS
    NS = TQ // OS
    NC = D // _LANES

    def out_prep(t, j):
        o = ot_ref[t, :, pl.ds(j * OS, OS)].T.astype(_BF16)
        on_ref[pl.ds((t * TQ + j * OS) // 2, OS // 2), :] = pltpu.bitcast(o, jnp.uint32)

    def out_piece(t, j, n):
        q0 = t * TQ + j * OS
        c0 = n * _LANES
        o = pltpu.bitcast(on_ref[pl.ds(q0 // 2, OS // 2), :], _BF16)
        attn = jnp.dot(o, wo_ref[:, c0:c0 + _LANES], preferred_element_type=_F32)
        xf = x_ref[pl.ds(q0, OS), c0:c0 + _LANES].astype(_F32)
        xnf = xn_ref[pl.ds(q0, OS), c0:c0 + _LANES].astype(_F32)
        ob_ref[t, pl.ds(j * OS, OS), c0:c0 + _LANES] = ((xf + attn) + xnf).astype(ob_ref.dtype)

    slices = [(t, j) for t in range(NQ - 1) for j in range(NS)]
    tasks = []
    for i, (t, j) in enumerate(slices):
        for n in range(NC):
            tk = [functools.partial(out_piece, t, j, n)]
            if n == 0 and i + 1 < len(slices):
                tk.append(functools.partial(out_prep, *slices[i + 1]))
            if n == NC - 1 and j == NS - 1:
                tk.append(lambda t=t: o_copy(t).start())
            tasks.append(tk)
    out_prep(*slices[0])
    n_side = min(len(tasks), G * NK - 1)
    side = {1 + (n * (G * NK - 1)) // n_side: tasks[n] for n in range(n_side)}
    block((NB - 1) * G, ms, do_a=False, side=side)
    for tk in tasks[n_side:]:
        for task in tk:
            task()
    for j in range(NS):
        out_prep(NQ - 1, j)
    for j in range(NS):
        for n in range(NC):
            out_piece(NQ - 1, j, n)
        o_copy_slice(j).start()
    for t in range(NQ - 1):
        o_copy(t).wait()
    for j in range(NS):
        o_copy_slice(j).wait()


@jax.jit
def pallas_parallel_sum__softmax_full_mha__moe_arch_mod__prompt_kernel(
    A_x: jax.Array,
    A_wqkv: jax.Array,
    A_wo: jax.Array,
    B_x: jax.Array,
    B_w_r: jax.Array,
    B_w_gate: jax.Array,
    B_w_up: jax.Array,
    B_w_down: jax.Array,
):
    B, S, D = A_x.shape
    assert B == 1
    F = B_w_gate.shape[1]
    TQ, TK, RB = _TQ, _TK, _RB
    NQ = S // TQ
    x2 = A_x.reshape(S, D)

    kern = functools.partial(_kernel, S=S, D=D, F=F, TQ=TQ, TK=TK, RB=RB)
    hbm = pl.BlockSpec(memory_space=pl.ANY)
    out = pl.pallas_call(
        kern,
        in_specs=[hbm, hbm, hbm, pl.BlockSpec(memory_space=pltpu.VMEM), hbm, hbm, hbm],
        out_specs=hbm,
        out_shape=jax.ShapeDtypeStruct((S, D), A_x.dtype),
        scratch_shapes=[
            pltpu.VMEM((S, D), _BF16),
            pltpu.VMEM((D, D), _BF16),
            pltpu.VMEM((D, D), _BF16),
            pltpu.VMEM((D, D), _BF16),
            pltpu.VMEM((D, D), _BF16),
            pltpu.VMEM((D, F), _BF16),
            pltpu.VMEM((D, F), _BF16),
            pltpu.VMEM((F, D), _BF16),
            pltpu.VMEM((2 * D + 16, D), _BF16),
            pltpu.VMEM((S, D), _BF16),
            pltpu.VMEM((D // 2, S), jnp.uint32),
            pltpu.VMEM((_H, S // 2, _LANES), jnp.uint32),
            pltpu.VMEM((D // 2, S), jnp.uint32),
            pltpu.VMEM((8, S), _F32),
            pltpu.VMEM((NQ, D, TQ), _F32),
            pltpu.VMEM((S // 2, D), jnp.uint32),
            pltpu.VMEM((NQ, TQ, D), _BF16),
            pltpu.SemaphoreType.DMA((7,)),
            pltpu.SemaphoreType.DMA((S // RB,)),
            pltpu.SemaphoreType.DMA((NQ - 1 + TQ // _OS,)),
        ] + [pltpu.VMEM((S, TQ), _F32) for _ in range(_G)],
        compiler_params=pltpu.CompilerParams(
            vmem_limit_bytes=96 * 1024 * 1024,
        ),
    )(x2, A_wqkv, A_wo, B_w_r, B_w_gate, B_w_up, B_w_down)
    return out.reshape(B, S, D)
```

```python
import functools
import math

import jax
import jax.numpy as jnp
import numpy as np
import jax.experimental.pallas as pl
import jax.experimental.pallas.tpu as pltpu

_H = 32
_LANES = 128
_TQ = 256
_TK = 128
_G = 8
_OS = 128
_RB = 256

_F32 = jnp.float32
_BF16 = jnp.bfloat16


def _bf(x):
    return x.astype(_BF16).astype(_F32)


def _kernel(x_hbm, wqkv_hbm, wo_hbm, wr_ref, wg_hbm, wu_hbm, wd_hbm,
            o_hbm,
            x_ref, wq_ref, wk_ref, wv_ref, wo_ref, wg_ref, wu_ref, wd_ref,
            wt_ref, xn_ref, qt_ref, kh_ref, vt_ref, r_ref, ot_ref,
            on_ref, ob_ref, sems, xsems, osems, *s_refs_all,
            S, D, F, TQ, TK, RB):
    H = _H
    DH = D // H
    HPG = _LANES // DH
    NK = S // TK
    NQ = S // TQ
    NRB = S // RB
    NITEMS = NQ * H

    def x_copy(i):
        return pltpu.make_async_copy(x_hbm.at[pl.ds(i * RB, RB), :],
                                     x_ref.at[pl.ds(i * RB, RB), :], xsems.at[i])

    cwq = pltpu.make_async_copy(wqkv_hbm.at[:, pl.ds(0, D)], wq_ref, sems.at[0])
    cwk = pltpu.make_async_copy(wqkv_hbm.at[:, pl.ds(D, D)], wk_ref, sems.at[1])
    cwv = pltpu.make_async_copy(wqkv_hbm.at[:, pl.ds(2 * D, D)], wv_ref, sems.at[2])
    co = pltpu.make_async_copy(wo_hbm, wo_ref, sems.at[3])
    cg = pltpu.make_async_copy(wg_hbm, wg_ref, sems.at[4])
    cu = pltpu.make_async_copy(wu_hbm, wu_ref, sems.at[5])
    cd = pltpu.make_async_copy(wd_hbm, wd_ref, sems.at[6])
    x_copy(0).start()
    cwk.start()
    cwq.start()
    cwv.start()
    for i in range(1, NRB):
        x_copy(i).start()

    eps_b = float(np.asarray(1e-5, dtype=jnp.bfloat16).astype(np.float32))
    qscale = (DH ** -0.5) * math.log2(math.e)

    def ln_rows(r0):
        xf = x_ref[pl.ds(r0, RB), :].astype(_F32)
        mean = jnp.sum(xf, axis=-1, keepdims=True) * (1.0 / D)
        cen = xf - mean
        var = jnp.sum(cen * cen, axis=-1, keepdims=True) * (1.0 / D)
        m_b = _bf(mean)
        v_b = _bf(var)
        d = _bf(xf - m_b)
        sd = _bf(jnp.sqrt(_bf(v_b + eps_b)))
        xn_ref[pl.ds(r0, RB), :] = (d / sd).astype(_BF16)

    def k_rows(r0):
        xn = xn_ref[pl.ds(r0, RB), :]
        kk = jnp.dot(xn, wk_ref[...], preferred_element_type=_F32).astype(_BF16)
        kw = pltpu.bitcast(kk, jnp.uint32)
        for gi in range(D // _LANES):
            kg = kw[:, gi * _LANES:(gi + 1) * _LANES]
            for j in range(HPG):
                kr = kg if j == 0 else pltpu.roll(kg, _LANES - j * DH, 1)
                kh_ref[gi * HPG + j, pl.ds(r0 // 2, RB // 2), :] = kr

    def qv_rows(r0):
        t = jax.lax.dot_general(wt_ref[...], xn_ref[pl.ds(r0, RB), :], (((1,), (1,)), ((), ())),
                                preferred_element_type=_F32)
        qt_ref[:, pl.ds(r0, RB)] = pltpu.bitcast((t[0:D, :] * qscale).astype(_BF16), jnp.uint32)
        vt_ref[:, pl.ds(r0, RB)] = pltpu.bitcast(t[D:2 * D, :].astype(_BF16), jnp.uint32)
        r_ref[:, pl.ds(r0, RB)] = _bf(t[2 * D:2 * D + 8, :])

    x_copy(0).wait()
    ln_rows(0)
    cwk.wait()
    cwq.wait()
    wt_ref[0:D, :] = wq_ref[...].astype(_F32).T.astype(_BF16)
    k_rows(0)
    cwv.wait()
    x_copy(1).wait()
    wt_ref[D:2 * D, :] = wv_ref[...].astype(_F32).T.astype(_BF16)
    wt_ref[2 * D:2 * D + 16, :] = jnp.broadcast_to(
        wr_ref[...].astype(_F32).reshape(1, D), (16, D)).astype(_BF16)
    ln_rows(RB)
    qv_rows(0)
    x_copy(2).wait()
    x_copy(3).wait()
    ln_rows(2 * RB)
    k_rows(RB)
    ln_rows(3 * RB)
    qv_rows(RB)
    for i in range(4, NRB):
        x_copy(i).wait()
    co.start()
    cg.start()
    cu.start()
    cd.start()
    for i in range(2, NRB):
        if i + 2 < NRB:
            ln_rows((i + 2) * RB)
        k_rows(i * RB)
        qv_rows(i * RB)

    rt = {}
    FC = 2 * _LANES
    NFC = F // FC

    def rt_select():
        r = r_ref[...]
        rmax = jnp.max(r, axis=1, keepdims=True)
        lane = jax.lax.broadcasted_iota(jnp.int32, (8, S), 1)
        idx = jnp.min(jnp.where(r == rmax, lane, S - 1))
        g0 = pl.multiple_of((idx // 16) * 16, 16)
        rt["g0"] = g0
        rt["sub"] = idx - g0
        rt["r_sel"] = _bf(jax.nn.sigmoid(rmax[0:1, :]))
        rt["x_sel"] = xn_ref[pl.ds(g0, 16), :]
        rt["y"] = jnp.zeros((16, D), _F32)

    def rt_ffn(i):
        c0 = i * FC
        g = _bf(jnp.dot(rt["x_sel"], wg_ref[:, c0:c0 + FC], preferred_element_type=_F32))
        g = _bf(g * jax.nn.sigmoid(g))
        u = _bf(jnp.dot(rt["x_sel"], wu_ref[:, c0:c0 + FC], preferred_element_type=_F32))
        rt["gu", i] = (g * u).astype(_BF16)

    def rt_down(i):
        c0 = i * FC
        rt["y"] = rt["y"] + jnp.dot(rt.pop(("gu", i)), wd_ref[c0:c0 + FC, :],
                                    preferred_element_type=_F32)

    def rt_final():
        sub = jax.lax.broadcasted_iota(jnp.int32, (16, D), 0)
        upd = jnp.where(sub == rt["sub"], _bf(_bf(rt["y"]) * rt["r_sel"]), 0.0)
        xn_ref[pl.ds(rt["g0"], 16), :] = (rt["x_sel"].astype(_F32) + upd).astype(_BF16)

    G = _G
    HW = DH // 2

    def stage_a(item, sref, kc, m8):
        h = item % H
        q0 = pl.multiple_of((item // H) * TQ, TQ)
        h0 = pl.multiple_of(h * HW, HW)
        k0 = kc * TK
        kc_blk = pltpu.bitcast(kh_ref[h, pl.ds(k0 // 2, TK // 2), :], _BF16)[:, 0:DH]
        qw = pltpu.bitcast(qt_ref[pl.ds(h0, HW), pl.ds(q0, TQ)], _BF16)
        s = jnp.dot(kc_blk, qw, preferred_element_type=_F32)
        sref[pl.ds(k0, TK), :] = s
        return jnp.maximum(m8, jnp.max(s.reshape(TK // 8, 8, TQ), axis=0))

    def stage_b(item, sref, kc, m, l8, acc):
        k0 = kc * TK
        h0 = pl.multiple_of((item % H) * HW, HW)
        pieces = []
        for r in range(TK // 16):
            pa = jnp.exp2(sref[pl.ds(k0 + 16 * r, 8), :] - m)
            pb = jnp.exp2(sref[pl.ds(k0 + 16 * r + 8, 8), :] - m)
            l8 = (l8 + pa) + pb
            pieces += [pa, pb]
        p = jnp.concatenate(pieces, axis=0).astype(_BF16)
        vw = pltpu.bitcast(vt_ref[pl.ds(h0, HW), pl.ds(k0, TK)], _BF16)
        acc = acc + jnp.dot(vw, p, preferred_element_type=_F32)
        return l8, acc

    def finish(item, l8, acc):
        qt = item // H
        h0 = pl.multiple_of((item % H) * DH, DH)
        l = jnp.sum(l8, axis=0, keepdims=True)
        ot_ref[qt, pl.ds(h0, DH), :] = acc / l

    neg = jnp.full((8, TQ), -jnp.inf, _F32)
    zl = jnp.zeros((8, TQ), _F32)
    za = jnp.zeros((DH, TQ), _F32)

    def bmax(m8):
        return jnp.broadcast_to(jnp.max(m8, axis=0, keepdims=True), (8, TQ))

    def block(base, ms, do_a=True, do_b=True, side=None):
        new_ms = []
        m8 = l8 = acc = None
        for t in range(G * NK):
            g, c = divmod(t, NK)
            if do_b:
                if c == 0:
                    if g == 0:
                        l8, acc = zl, za
                    else:
                        l8, acc = jnp.minimum(l8, 0.0), jnp.minimum(jnp.abs(acc), 0.0)
                l8, acc = stage_b(base + g, s_refs_all[g], c, ms[g], l8, acc)
                if c == NK - 1:
                    finish(base + g, l8, acc)
            if do_a:
                if c == 0:
                    m8 = neg
                m8 = stage_a(base + G + g, s_refs_all[g], c, m8)
                if c == NK - 1:
                    new_ms.append(bmax(m8))
            if side is not None:
                for task in side.get(t, ()):
                    task()
        return tuple(new_ms)

    NB = NITEMS // G
    cg.wait()
    cu.wait()
    cd.wait()
    side = {0: [rt_select]}
    stride = (G * NK - 4) // (NFC + 1)
    for i in range(NFC):
        side.setdefault(2 + i * stride, []).append(functools.partial(rt_ffn, i))
        side.setdefault(2 + (i + 1) * stride, []).append(functools.partial(rt_down, i))
    side.setdefault(G * NK - 1, []).append(rt_final)
    ms = block(-G, None, do_b=False, side=side)

    ms = jax.lax.fori_loop(0, NB - 1, lambda j, ms: block(j * G, ms), ms)

    co.wait()

    def o_copy(t):
        return pltpu.make_async_copy(ob_ref.at[t], o_hbm.at[pl.ds(t * TQ, TQ), :], osems.at[t])

    def o_copy_slice(j):
        t = NQ - 1
        return pltpu.make_async_copy(ob_ref.at[t, pl.ds(j * _OS, _OS), :],
                                     o_hbm.at[pl.ds(t * TQ + j * _OS, _OS), :], osems.at[t + j])

    OS = _OS
    NS = TQ // OS
    NC = D // _LANES

    def out_prep(t, j):
        o = ot_ref[t, :, pl.ds(j * OS, OS)].T.astype(_BF16)
        on_ref[pl.ds((t * TQ + j * OS) // 2, OS // 2), :] = pltpu.bitcast(o, jnp.uint32)

    def out_piece(t, j, n):
        q0 = t * TQ + j * OS
        c0 = n * _LANES
        o = pltpu.bitcast(on_ref[pl.ds(q0 // 2, OS // 2), :], _BF16)
        attn = jnp.dot(o, wo_ref[:, c0:c0 + _LANES], preferred_element_type=_F32)
        xf = x_ref[pl.ds(q0, OS), c0:c0 + _LANES].astype(_F32)
        xnf = xn_ref[pl.ds(q0, OS), c0:c0 + _LANES].astype(_F32)
        ob_ref[t, pl.ds(j * OS, OS), c0:c0 + _LANES] = ((xf + attn) + xnf).astype(ob_ref.dtype)

    slices = [(t, j) for t in range(NQ - 1) for j in range(NS)]
    tasks = []
    for i, (t, j) in enumerate(slices):
        for n in range(NC):
            tk = [functools.partial(out_piece, t, j, n)]
            if n == 0 and i + 1 < len(slices):
                tk.append(functools.partial(out_prep, *slices[i + 1]))
            if n == NC - 1 and j == NS - 1:
                tk.append(lambda t=t: o_copy(t).start())
            tasks.append(tk)
    out_prep(*slices[0])
    n_side = min(len(tasks), G * NK - 1)
    side = {1 + (n * (G * NK - 1)) // n_side: tasks[n] for n in range(n_side)}
    block((NB - 1) * G, ms, do_a=False, side=side)
    for tk in tasks[n_side:]:
        for task in tk:
            task()
    for j in range(NS):
        out_prep(NQ - 1, j)
    for j in range(NS):
        for n in range(NC):
            out_piece(NQ - 1, j, n)
        o_copy_slice(j).start()
    for t in range(NQ - 1):
        o_copy(t).wait()
    for j in range(NS):
        o_copy_slice(j).wait()


@jax.jit
def pallas_parallel_sum__softmax_full_mha__moe_arch_mod__prompt_kernel(
    A_x: jax.Array,
    A_wqkv: jax.Array,
    A_wo: jax.Array,
    B_x: jax.Array,
    B_w_r: jax.Array,
    B_w_gate: jax.Array,
    B_w_up: jax.Array,
    B_w_down: jax.Array,
):
    B, S, D = A_x.shape
    assert B == 1
    F = B_w_gate.shape[1]
    TQ, TK, RB = _TQ, _TK, _RB
    NQ = S // TQ
    x2 = A_x.reshape(S, D)

    kern = functools.partial(_kernel, S=S, D=D, F=F, TQ=TQ, TK=TK, RB=RB)
    hbm = pl.BlockSpec(memory_space=pl.ANY)
    out = pl.pallas_call(
        kern,
        in_specs=[hbm, hbm, hbm, pl.BlockSpec(memory_space=pltpu.VMEM), hbm, hbm, hbm],
        out_specs=hbm,
        out_shape=jax.ShapeDtypeStruct((S, D), A_x.dtype),
        scratch_shapes=[
            pltpu.VMEM((S, D), _BF16),
            pltpu.VMEM((D, D), _BF16),
            pltpu.VMEM((D, D), _BF16),
            pltpu.VMEM((D, D), _BF16),
            pltpu.VMEM((D, D), _BF16),
            pltpu.VMEM((D, F), _BF16),
            pltpu.VMEM((D, F), _BF16),
            pltpu.VMEM((F, D), _BF16),
            pltpu.VMEM((2 * D + 16, D), _BF16),
            pltpu.VMEM((S, D), _BF16),
            pltpu.VMEM((D // 2, S), jnp.uint32),
            pltpu.VMEM((_H, S // 2, _LANES), jnp.uint32),
            pltpu.VMEM((D // 2, S), jnp.uint32),
            pltpu.VMEM((8, S), _F32),
            pltpu.VMEM((NQ, D, TQ), _F32),
            pltpu.VMEM((S // 2, D), jnp.uint32),
            pltpu.VMEM((NQ, TQ, D), _BF16),
            pltpu.SemaphoreType.DMA((7,)),
            pltpu.SemaphoreType.DMA((S // RB,)),
            pltpu.SemaphoreType.DMA((NQ - 1 + TQ // _OS,)),
        ] + [pltpu.VMEM((S, TQ), _F32) for _ in range(_G)],
        compiler_params=pltpu.CompilerParams(
            vmem_limit_bytes=96 * 1024 * 1024,
        ),
    )(x2, A_wqkv, A_wo, B_w_r, B_w_gate, B_w_up, B_w_down)
    return out.reshape(B, S, D)
```

```python
import functools
import math

import jax
import jax.numpy as jnp
import numpy as np
import jax.experimental.pallas as pl
import jax.experimental.pallas.tpu as pltpu

_H = 32
_LANES = 128
_TQ = 256
_TK = 128
_G = 8
_OS = 128
_RB = 256

_F32 = jnp.float32
_BF16 = jnp.bfloat16


def _bf(x):
    return x.astype(_BF16).astype(_F32)


def _kernel(x_hbm, wqkv_hbm, wo_hbm, wr_hbm, wg_hbm, wu_hbm, wd_hbm,
            o_hbm,
            x_ref, wq_ref, wk_ref, wv_ref, wo_ref, wr_ref, wg_ref, wu_ref, wd_ref,
            wt_ref, xn_ref, qt_ref, kh_ref, vt_ref, r_ref, ot_ref,
            on_ref, ob_ref, sems, xsems, osems, *s_refs_all,
            S, D, F, TQ, TK, RB):
    H = _H
    DH = D // H
    HPG = _LANES // DH
    NK = S // TK
    NQ = S // TQ
    NRB = S // RB
    NITEMS = NQ * H

    def x_copy(i):
        return pltpu.make_async_copy(x_hbm.at[pl.ds(i * RB, RB), :],
                                     x_ref.at[pl.ds(i * RB, RB), :], xsems.at[i])

    cwq = pltpu.make_async_copy(wqkv_hbm.at[:, pl.ds(0, D)], wq_ref, sems.at[0])
    cwk = pltpu.make_async_copy(wqkv_hbm.at[:, pl.ds(D, D)], wk_ref, sems.at[1])
    cwv = pltpu.make_async_copy(wqkv_hbm.at[:, pl.ds(2 * D, D)], wv_ref, sems.at[2])
    co = pltpu.make_async_copy(wo_hbm, wo_ref, sems.at[3])
    cg = pltpu.make_async_copy(wg_hbm, wg_ref, sems.at[4])
    cu = pltpu.make_async_copy(wu_hbm, wu_ref, sems.at[5])
    cd = pltpu.make_async_copy(wd_hbm, wd_ref, sems.at[6])
    cr = pltpu.make_async_copy(wr_hbm, wr_ref, sems.at[7])
    x_copy(0).start()
    cwk.start()
    cwq.start()
    cwv.start()
    cr.start()
    for i in range(1, NRB):
        x_copy(i).start()

    eps_b = float(np.asarray(1e-5, dtype=jnp.bfloat16).astype(np.float32))
    qscale = (DH ** -0.5) * math.log2(math.e)

    def ln_rows(r0):
        xf = x_ref[pl.ds(r0, RB), :].astype(_F32)
        mean = jnp.sum(xf, axis=-1, keepdims=True) * (1.0 / D)
        cen = xf - mean
        var = jnp.sum(cen * cen, axis=-1, keepdims=True) * (1.0 / D)
        m_b = _bf(mean)
        v_b = _bf(var)
        d = _bf(xf - m_b)
        sd = _bf(jnp.sqrt(_bf(v_b + eps_b)))
        xn_ref[pl.ds(r0, RB), :] = (d / sd).astype(_BF16)

    def k_rows(r0):
        xn = xn_ref[pl.ds(r0, RB), :]
        kk = jnp.dot(xn, wk_ref[...], preferred_element_type=_F32).astype(_BF16)
        kw = pltpu.bitcast(kk, jnp.uint32)
        for gi in range(D // _LANES):
            kg = kw[:, gi * _LANES:(gi + 1) * _LANES]
            for j in range(HPG):
                kr = kg if j == 0 else pltpu.roll(kg, _LANES - j * DH, 1)
                kh_ref[gi * HPG + j, pl.ds(r0 // 2, RB // 2), :] = kr

    def qv_rows(r0):
        t = jax.lax.dot_general(wt_ref[...], xn_ref[pl.ds(r0, RB), :], (((1,), (1,)), ((), ())),
                                preferred_element_type=_F32)
        qt_ref[:, pl.ds(r0, RB)] = pltpu.bitcast((t[0:D, :] * qscale).astype(_BF16), jnp.uint32)
        vt_ref[:, pl.ds(r0, RB)] = pltpu.bitcast(t[D:2 * D, :].astype(_BF16), jnp.uint32)
        r_ref[:, pl.ds(r0, RB)] = _bf(t[2 * D:2 * D + 8, :])

    x_copy(0).wait()
    ln_rows(0)
    cwk.wait()
    cwq.wait()
    wt_ref[0:D, :] = wq_ref[...].astype(_F32).T.astype(_BF16)
    k_rows(0)
    cwv.wait()
    cr.wait()
    x_copy(1).wait()
    wt_ref[D:2 * D, :] = wv_ref[...].astype(_F32).T.astype(_BF16)
    wt_ref[2 * D:2 * D + 16, :] = jnp.broadcast_to(
        wr_ref[...].astype(_F32).reshape(1, D), (16, D)).astype(_BF16)
    ln_rows(RB)
    qv_rows(0)
    x_copy(2).wait()
    x_copy(3).wait()
    ln_rows(2 * RB)
    k_rows(RB)
    ln_rows(3 * RB)
    qv_rows(RB)
    for i in range(4, NRB):
        x_copy(i).wait()
    co.start()
    cg.start()
    cu.start()
    cd.start()
    for i in range(2, NRB):
        if i + 2 < NRB:
            ln_rows((i + 2) * RB)
        k_rows(i * RB)
        qv_rows(i * RB)

    rt = {}
    FC = 2 * _LANES
    NFC = F // FC

    def rt_select():
        r = r_ref[...]
        rmax = jnp.max(r, axis=1, keepdims=True)
        lane = jax.lax.broadcasted_iota(jnp.int32, (8, S), 1)
        idx = jnp.min(jnp.where(r == rmax, lane, S - 1))
        g0 = pl.multiple_of((idx // 16) * 16, 16)
        rt["g0"] = g0
        rt["sub"] = idx - g0
        rt["r_sel"] = _bf(jax.nn.sigmoid(rmax[0:1, :]))
        rt["x_sel"] = xn_ref[pl.ds(g0, 16), :]
        rt["y"] = jnp.zeros((16, D), _F32)

    def rt_ffn(i):
        c0 = i * FC
        g = _bf(jnp.dot(rt["x_sel"], wg_ref[:, c0:c0 + FC], preferred_element_type=_F32))
        g = _bf(g * jax.nn.sigmoid(g))
        u = _bf(jnp.dot(rt["x_sel"], wu_ref[:, c0:c0 + FC], preferred_element_type=_F32))
        rt["gu", i] = (g * u).astype(_BF16)

    def rt_down(i):
        c0 = i * FC
        rt["y"] = rt["y"] + jnp.dot(rt.pop(("gu", i)), wd_ref[c0:c0 + FC, :],
                                    preferred_element_type=_F32)

    def rt_final():
        sub = jax.lax.broadcasted_iota(jnp.int32, (16, D), 0)
        upd = jnp.where(sub == rt["sub"], _bf(_bf(rt["y"]) * rt["r_sel"]), 0.0)
        xn_ref[pl.ds(rt["g0"], 16), :] = (rt["x_sel"].astype(_F32) + upd).astype(_BF16)

    G = _G
    HW = DH // 2

    def stage_a(item, sref, kc, m8):
        h = item % H
        q0 = pl.multiple_of((item // H) * TQ, TQ)
        h0 = pl.multiple_of(h * HW, HW)
        k0 = kc * TK
        kc_blk = pltpu.bitcast(kh_ref[h, pl.ds(k0 // 2, TK // 2), :], _BF16)[:, 0:DH]
        qw = pltpu.bitcast(qt_ref[pl.ds(h0, HW), pl.ds(q0, TQ)], _BF16)
        s = jnp.dot(kc_blk, qw, preferred_element_type=_F32)
        sref[pl.ds(k0, TK), :] = s
        return jnp.maximum(m8, jnp.max(s.reshape(TK // 8, 8, TQ), axis=0))

    def stage_b(item, sref, kc, m, l8, acc):
        k0 = kc * TK
        h0 = pl.multiple_of((item % H) * HW, HW)
        pieces = []
        for r in range(TK // 16):
            pa = jnp.exp2(sref[pl.ds(k0 + 16 * r, 8), :] - m)
            pb = jnp.exp2(sref[pl.ds(k0 + 16 * r + 8, 8), :] - m)
            l8 = (l8 + pa) + pb
            pieces += [pa, pb]
        p = jnp.concatenate(pieces, axis=0).astype(_BF16)
        vw = pltpu.bitcast(vt_ref[pl.ds(h0, HW), pl.ds(k0, TK)], _BF16)
        acc = acc + jnp.dot(vw, p, preferred_element_type=_F32)
        return l8, acc

    def finish(item, l8, acc):
        qt = item // H
        h0 = pl.multiple_of((item % H) * DH, DH)
        l = jnp.sum(l8, axis=0, keepdims=True)
        ot_ref[qt, pl.ds(h0, DH), :] = acc / l

    neg = jnp.full((8, TQ), -jnp.inf, _F32)
    zl = jnp.zeros((8, TQ), _F32)
    za = jnp.zeros((DH, TQ), _F32)

    def bmax(m8):
        return jnp.broadcast_to(jnp.max(m8, axis=0, keepdims=True), (8, TQ))

    def block(base, ms, do_a=True, do_b=True, side=None):
        new_ms = []
        m8 = l8 = acc = None
        for t in range(G * NK):
            g, c = divmod(t, NK)
            if do_b:
                if c == 0:
                    if g == 0:
                        l8, acc = zl, za
                    else:
                        l8, acc = jnp.minimum(l8, 0.0), jnp.minimum(jnp.abs(acc), 0.0)
                l8, acc = stage_b(base + g, s_refs_all[g], c, ms[g], l8, acc)
                if c == NK - 1:
                    finish(base + g, l8, acc)
            if do_a:
                if c == 0:
                    m8 = neg
                m8 = stage_a(base + G + g, s_refs_all[g], c, m8)
                if c == NK - 1:
                    new_ms.append(bmax(m8))
            if side is not None:
                for task in side.get(t, ()):
                    task()
        return tuple(new_ms)

    NB = NITEMS // G
    cg.wait()
    cu.wait()
    cd.wait()
    side = {0: [rt_select]}
    stride = (G * NK - 4) // (NFC + 1)
    for i in range(NFC):
        side.setdefault(2 + i * stride, []).append(functools.partial(rt_ffn, i))
        side.setdefault(2 + (i + 1) * stride, []).append(functools.partial(rt_down, i))
    side.setdefault(G * NK - 1, []).append(rt_final)
    ms = block(-G, None, do_b=False, side=side)

    ms = jax.lax.fori_loop(0, NB - 1, lambda j, ms: block(j * G, ms), ms)

    co.wait()

    def o_copy(t):
        return pltpu.make_async_copy(ob_ref.at[t], o_hbm.at[pl.ds(t * TQ, TQ), :], osems.at[t])

    def o_copy_slice(j):
        t = NQ - 1
        return pltpu.make_async_copy(ob_ref.at[t, pl.ds(j * _OS, _OS), :],
                                     o_hbm.at[pl.ds(t * TQ + j * _OS, _OS), :], osems.at[t + j])

    OS = _OS
    NS = TQ // OS
    NC = D // _LANES

    def out_prep(t, j):
        o = ot_ref[t, :, pl.ds(j * OS, OS)].T.astype(_BF16)
        on_ref[pl.ds((t * TQ + j * OS) // 2, OS // 2), :] = pltpu.bitcast(o, jnp.uint32)

    def out_piece(t, j, n):
        q0 = t * TQ + j * OS
        c0 = n * _LANES
        o = pltpu.bitcast(on_ref[pl.ds(q0 // 2, OS // 2), :], _BF16)
        attn = jnp.dot(o, wo_ref[:, c0:c0 + _LANES], preferred_element_type=_F32)
        xf = x_ref[pl.ds(q0, OS), c0:c0 + _LANES].astype(_F32)
        xnf = xn_ref[pl.ds(q0, OS), c0:c0 + _LANES].astype(_F32)
        ob_ref[t, pl.ds(j * OS, OS), c0:c0 + _LANES] = ((xf + attn) + xnf).astype(ob_ref.dtype)

    slices = [(t, j) for t in range(NQ - 1) for j in range(NS)]
    tasks = []
    for i, (t, j) in enumerate(slices):
        for n in range(NC):
            tk = [functools.partial(out_piece, t, j, n)]
            if n == 0 and i + 1 < len(slices):
                tk.append(functools.partial(out_prep, *slices[i + 1]))
            if n == NC - 1 and j == NS - 1:
                tk.append(lambda t=t: o_copy(t).start())
            tasks.append(tk)
    out_prep(*slices[0])
    n_side = min(len(tasks), G * NK - 1)
    side = {1 + (n * (G * NK - 1)) // n_side: tasks[n] for n in range(n_side)}
    block((NB - 1) * G, ms, do_a=False, side=side)
    for tk in tasks[n_side:]:
        for task in tk:
            task()
    for j in range(NS):
        out_prep(NQ - 1, j)
    for j in range(NS):
        for n in range(NC):
            out_piece(NQ - 1, j, n)
        o_copy_slice(j).start()
    for t in range(NQ - 1):
        o_copy(t).wait()
    for j in range(NS):
        o_copy_slice(j).wait()


@jax.jit
def pallas_parallel_sum__softmax_full_mha__moe_arch_mod__prompt_kernel(
    A_x: jax.Array,
    A_wqkv: jax.Array,
    A_wo: jax.Array,
    B_x: jax.Array,
    B_w_r: jax.Array,
    B_w_gate: jax.Array,
    B_w_up: jax.Array,
    B_w_down: jax.Array,
):
    B, S, D = A_x.shape
    assert B == 1
    F = B_w_gate.shape[1]
    TQ, TK, RB = _TQ, _TK, _RB
    NQ = S // TQ
    x2 = A_x.reshape(S, D)

    kern = functools.partial(_kernel, S=S, D=D, F=F, TQ=TQ, TK=TK, RB=RB)
    hbm = pl.BlockSpec(memory_space=pl.ANY)
    out = pl.pallas_call(
        kern,
        in_specs=[hbm] * 7,
        out_specs=hbm,
        out_shape=jax.ShapeDtypeStruct((S, D), A_x.dtype),
        scratch_shapes=[
            pltpu.VMEM((S, D), _BF16),
            pltpu.VMEM((D, D), _BF16),
            pltpu.VMEM((D, D), _BF16),
            pltpu.VMEM((D, D), _BF16),
            pltpu.VMEM((D, D), _BF16),
            pltpu.VMEM((D,), _BF16),
            pltpu.VMEM((D, F), _BF16),
            pltpu.VMEM((D, F), _BF16),
            pltpu.VMEM((F, D), _BF16),
            pltpu.VMEM((2 * D + 16, D), _BF16),
            pltpu.VMEM((S, D), _BF16),
            pltpu.VMEM((D // 2, S), jnp.uint32),
            pltpu.VMEM((_H, S // 2, _LANES), jnp.uint32),
            pltpu.VMEM((D // 2, S), jnp.uint32),
            pltpu.VMEM((8, S), _F32),
            pltpu.VMEM((NQ, D, TQ), _F32),
            pltpu.VMEM((S // 2, D), jnp.uint32),
            pltpu.VMEM((NQ, TQ, D), _BF16),
            pltpu.SemaphoreType.DMA((8,)),
            pltpu.SemaphoreType.DMA((S // RB,)),
            pltpu.SemaphoreType.DMA((NQ - 1 + TQ // _OS,)),
        ] + [pltpu.VMEM((S, TQ), _F32) for _ in range(_G)],
        compiler_params=pltpu.CompilerParams(
            vmem_limit_bytes=96 * 1024 * 1024,
        ),
    )(x2, A_wqkv, A_wo, B_w_r, B_w_gate, B_w_up, B_w_down)
    return out.reshape(B, S, D)
```
